```python
import os as _os
_os.environ.setdefault("JAX_PLATFORMS", "cpu")
import jax
import jax.numpy as jnp

def _softmax(x, axis=-1):
    return jax.nn.softmax(x, axis=axis)
def _gelu(x):
    return jax.nn.gelu(x, approximate=True)
def _silu(x):
    return jax.nn.silu(x)
def _sigmoid(x):
    return jax.nn.sigmoid(x)
def _layernorm(x, axis=-1, eps=1e-5):
    m = jnp.mean(x, axis=axis, keepdims=True)
    v = jnp.var(x, axis=axis, keepdims=True)
    return (x - m) / jnp.sqrt(v + eps)
def _scatter_add(tgt, idx, src, axis=0):
    return tgt.at[idx].add(src)
def _segment_sum(src, seg, n):
    return jax.ops.segment_sum(src, seg, n)
class _Rng:
    def __init__(self, key):
        self._k = key
    def _next(self):
        self._k, sub = jax.random.split(self._k)
        return sub
    def normal(self, shape):
        return jax.random.normal(self._next(), shape, dtype=jnp.bfloat16)
    def randint(self, lo, hi, shape):
        return jax.random.randint(self._next(), shape, lo, hi, dtype=jnp.int32)
    def uniform(self, shape, lo=0.0, hi=1.0):
        return jax.random.uniform(self._next(), shape, jnp.bfloat16, lo, hi)
    def permutation(self, n):
        return jax.random.permutation(self._next(), n)


kernel_name = 'sequential_preLN__linear_kernel_hedgehog__geglu_ffn__prompt'

def setup_inputs():
    _rng = _Rng(jax.random.key(int.from_bytes(__import__("os").urandom(4), "little")))
    _w = (lambda a: (lambda t: t.astype(jnp.bfloat16) if jnp.issubdtype(t.dtype, jnp.floating) else t)(jnp.asarray(a)))
    def _A_setup():
        B, S, D, H = 1, 2048, 640, 32
        Dh = D // H
        return {
            "x": _w((lambda *s: _rng.normal(s) * 0.05)(B, S, D)),
            "wqkv": _w((lambda *s: _rng.normal(s) * 0.2)(D, 3 * D)),
            "w_phi": _w((lambda *s: _rng.normal(s) * 0.2)(H, Dh, Dh) * (Dh ** -0.5)),
            "wo": _w((lambda *s: _rng.normal(s) * 0.05)(D, D)),
        }
    _A_in = _A_setup()

    def _B_setup():
        B, S, D, F = 1, 2048, 640, 1536
        return {
            "x": _w((lambda *s: _rng.normal(s) * 0.05)(B, S, D)),
            "w_gate": _w((lambda *s: _rng.normal(s) * 0.05)(D, F)),
            "w_up": _w((lambda *s: _rng.normal(s) * 0.05)(D, F)),
            "w_down": _w((lambda *s: _rng.normal(s) * 0.05)(F, D)),
        }
    _B_in = _B_setup()

    return {
        "A_x": _A_in["x"],
        "A_wqkv": _A_in["wqkv"],
        "A_w_phi": _A_in["w_phi"],
        "A_wo": _A_in["wo"],
        "B_x": _B_in["x"],
        "B_w_gate": _B_in["w_gate"],
        "B_w_up": _B_in["w_up"],
        "B_w_down": _B_in["w_down"],
    }

def reference(A_x, A_wqkv, A_w_phi, A_wo, B_x, B_w_gate, B_w_up, B_w_down):
    def _A_ref(x, wqkv, w_phi, wo):
        B, S, D = x.shape
        H = 32; Dh = D // H
        qkv = (lambda x, *d: x.transpose(*d))((x @ wqkv).reshape(B, S, 3, H, Dh), 2, 0, 3, 1, 4)
        q, k, v = qkv[0], qkv[1], qkv[2]
        pq = jnp.einsum("bhsd,hdf->bhsf", q, w_phi)
        pk = jnp.einsum("bhsd,hdf->bhsf", k, w_phi)
        phi_q = jnp.concatenate([_softmax(pq, axis=-1), _softmax(-pq, axis=-1)], axis=-1)
        phi_k = jnp.concatenate([_softmax(pk, axis=-1), _softmax(-pk, axis=-1)], axis=-1)
        kv = jnp.einsum("bhsf,bhsd->bhfd", phi_k, v)
        z  = jnp.einsum("bhsf->bhf", phi_k)
        num = jnp.einsum("bhqf,bhfd->bhqd", phi_q, kv)
        den = jnp.einsum("bhqf,bhf->bhq", phi_q, z)[..., None] + 1e-6
        o = num / den
        return (lambda x, *d: x.transpose(*d))(o, 0, 2, 1, 3).reshape(B, S, D) @ wo

    def _B_ref(x, w_gate, w_up, w_down):
        return (_gelu(x @ w_gate) * (x @ w_up)) @ w_down

    x = A_x
    h = x + _A_ref(_layernorm(x, axis=-1), A_wqkv, A_w_phi, A_wo)
    h2 = h + _B_ref(_layernorm(h, axis=-1), B_w_gate, B_w_up, B_w_down)
    return h2
```

```python
import math

import jax
import jax.numpy as jnp
from jax import lax
import jax.experimental.pallas as pl
import jax.experimental.pallas.tpu as pltpu

F32 = jnp.float32
BF16 = jnp.bfloat16

H = 32
LN_EPS = 1e-5
DEN_EPS = 1e-6
LOG2E = math.log2(math.e)

TS = 512
HM = TS // 2
KH = 256
LNR = 32
SP = (4, 8)
SWO = 1
GU = 0
ORD = 0
WVS = 1

_reciprocal = pltpu.reciprocal if hasattr(pltpu, "reciprocal") else pl.reciprocal
_NT = (((1,), (1,)), ((), ()))
_TN = (((0,), (0,)), ((), ()))


def _dot(a, b, dims=None):
    if dims is None:
        return jnp.dot(a, b, preferred_element_type=F32)
    return lax.dot_general(a, b, dims, preferred_element_type=F32)


def _b(t):
    return t.astype(BF16)


def _iota(shape, axis):
    return lax.broadcasted_iota(jnp.int32, shape, axis)


def _layernorm(x):
    out = []
    for r in range(0, x.shape[0], LNR):
        t = x[r:r + LNR].astype(F32)
        c = t - jnp.mean(t, axis=-1, keepdims=True)
        v = jnp.mean(c * c, axis=-1, keepdims=True)
        out.append(c * lax.rsqrt(v + LN_EPS))
    return jnp.concatenate(out, axis=0)


def _recip(s):
    r = _reciprocal(s, approx=True)
    return r * (2.0 - s * r)


def _reduce_f(rows, op):
    r = rows[0]
    for a in rows[1:]:
        r = op(r, a)
    r = op(r, pltpu.roll(r, 2, 0))
    return op(r, pltpu.roll(r, 4, 0))


def _dual_softmax(p):
    rows = [p[j * 8:(j + 1) * 8] for j in range(p.shape[0] // 8)]
    mx = _reduce_f(rows, jnp.maximum)
    mn = _reduce_f(rows, jnp.minimum)
    ep = [jnp.exp2(r - mx) for r in rows]
    en = [jnp.exp2(mn - r) for r in rows]
    rp = _recip(_reduce_f(ep, jnp.add))
    rn = _recip(_reduce_f(en, jnp.add))
    return jnp.concatenate([e * rp for e in ep] + [e * rn for e in en], axis=0)


def _geglu(g, u):
    c = math.sqrt(2.0 / math.pi)
    t = jnp.tanh(g * (c + (0.044715 * c) * (g * g)))
    return (g * (0.5 * u)) * (1.0 + t)


def _lhs_sums(a11, a12, a21, a22):
    return _b(a11 + a22), _b(a21 + a22), _b(a11 + a12), _b(a21 - a11), _b(a12 - a22)


def _rhs_sums(b11, b12, b21, b22):
    return _b(b11 + b22), _b(b12 - b22), _b(b21 - b11), _b(b11 + b12), _b(b21 + b22)


def _kernel(x_hbm, wqkv_hbm, wphi_hbm, wo_hbm, wg_hbm, wu_hbm, wd_hbm, out_hbm,
            x_v, wqkv_v, wphi_v, wo_v, wg_v, wu_v, wd_v, out_v,
            gu_v, dn_v, os_v, wt_v, ws_v, pt_v, y_v, ys_v, vt_v, zero_v, phiq_v, kv_v, kvb_v, sem_i, sem_o):
    S, D = x_v.shape
    F = wg_v.shape[1]
    HF = F // 2
    DH = D // H
    NG = H // 2
    GW = 2 * DH
    MV = GW + 8
    NT = S // TS
    K2 = 2 * KH

    x_chunks = [(0, HM), (HM, HM)] + [(i * TS, TS) for i in range(1, NT)]
    nx = len(x_chunks)

    def x_copy(n):
        r0, rows = x_chunks[n]
        return pltpu.make_async_copy(x_hbm.at[pl.ds(r0, rows)], x_v.at[pl.ds(r0, rows)], sem_i.at[7 + n])

    def wqkv_copy(j):
        return pltpu.make_async_copy(wqkv_hbm.at[:, pl.ds(j * D, D)], wqkv_v.at[j], sem_i.at[j])

    def wv_copy(c):
        n = D // WVS
        return pltpu.make_async_copy(wqkv_hbm.at[:, pl.ds(2 * D + c * n, n)], wqkv_v.at[2, :, pl.ds(c * n, n)],
                                     sem_i.at[8 + nx + c])

    def wd_copy(i):
        rows = pl.ds(i * (HF // NT), HF // NT)
        return pltpu.make_async_copy(wd_hbm.at[:, rows], wd_v.at[:, rows], sem_i.at[13 + nx + i])

    wo_copy = pltpu.make_async_copy(wo_hbm, wo_v, sem_i.at[3])
    wg_copy = pltpu.make_async_copy(wg_hbm, wg_v, sem_i.at[4])
    wu_copy = pltpu.make_async_copy(wu_hbm, wu_v, sem_i.at[5])
    wphi_copy = pltpu.make_async_copy(wphi_hbm, wphi_v, sem_i.at[6])

    wphi_copy.start()
    for c in range(WVS):
        wv_copy(c).start()
    for n in range(nx):
        x_copy(n).start()
    wqkv_copy(1).start()
    wqkv_copy(0).start()
    wo_copy.start()
    wg_copy.start()
    wu_copy.start()
    for i in range(NT):
        wd_copy(i).start()

    src = _iota((D, 128), 0)
    dst = (src & (H - 1)) * DH + (src >> 5)
    lane = _iota((D, 128), 1)
    wphi_copy.wait()
    wcat = jnp.concatenate([wphi_v[d] for d in range(DH)], axis=1)
    BW = 4 * GW
    rr = _iota((BW, 128), 0)
    cc = _iota((BW, 128), 1)
    pair = rr // GW
    feat = (rr - pair * GW) >> 1
    first = (2 * pair + (rr & 1)) * DH
    expand = _b(jnp.where(feat == cc, 1.0, 0.0))[:, :DH]
    for j in range(D // 128):
        w2t = _b(_dot(wcat, _b(jnp.where(dst == lane + 128 * j, 1.0, 0.0))))
        d_of_col = cc + (128 - 3 * GW) * j - first
        pt_v[j] = _b(jnp.where((d_of_col >= 0) & (d_of_col < DH), _dot(expand, w2t), 0.0))
    kv_v[...] = jnp.zeros(kv_v.shape, F32)
    zero_v[...] = jnp.zeros(zero_v.shape, jnp.int32)

    def ln_half(r0):
        y = _layernorm(x_v[r0:r0 + HM, :])
        y_v[r0:r0 + HM, :] = _b(y)
        return y

    def store_sums(i, y1, y2):
        for n, t in enumerate(_rhs_sums(y1[:, :KH], y2[:, :KH], y1[:, KH:K2], y2[:, KH:K2])):
            ys_v[i, n] = t

    def v_proj(r0, y, c, nc):
        rows = y.shape[0]
        gs = NG // nc
        vt = _dot(wt_v[2, c * gs * GW:(c + 1) * gs * GW, :], y, _NT)
        ones = jnp.ones((8, rows), F32)
        for g in range(gs):
            vt_v[r0 // TS, c * gs + g, :, r0 % TS:r0 % TS + rows] = _b(jnp.concatenate(
                [vt[g * GW:(g + 1) * GW], ones], axis=0))

    for c in range(WVS):
        wv_copy(c).wait()
        wt_v[2, c * (D // WVS):(c + 1) * (D // WVS), :] = wqkv_v[2, :, c * (D // WVS):(c + 1) * (D // WVS)].T
    x_copy(0).wait()
    y1 = ln_half(0)
    x_copy(1).wait()
    v_proj(0, _b(y1), 0, 1)
    y2 = ln_half(HM)
    v_proj(HM, _b(y2), 0, 1)
    store_sums(0, y1, y2)
    for n in range(2, nx):
        x_copy(n).wait()
    y1, y2 = ln_half(TS), ln_half(TS + HM)
    store_sums(1, y1, y2)
    for i in range(2, NT):
        cur = jnp.concatenate([_b(y1), _b(y2)], axis=0)
        y1 = ln_half(i * TS)
        v_proj((i - 1) * TS, cur, 0, 2)
        y2 = ln_half(i * TS + HM)
        store_sums(i, y1, y2)
        v_proj((i - 1) * TS, cur, 1, 2)
    wqkv_copy(1).wait()
    wqkv_copy(0).wait()
    v_proj((NT - 1) * TS, jnp.concatenate([_b(y1), _b(y2)], axis=0), 0, 1)

    def fold(j):
        blocks, tail = [], None
        for c in range(D // 128):
            r = _dot(pt_v[c], wqkv_v[j, :, 128 * c:128 * (c + 1)], _NT)
            blocks += [r[:GW] if tail is None else r[:GW] + tail, r[GW:3 * GW]]
            tail = r[3 * GW:]
        w = jnp.concatenate(blocks + [tail], axis=0) * LOG2E
        wt_v[j] = _b(w)
        return w

    wk, wq = fold(1), fold(0)
    for n, t in enumerate(_lhs_sums(wq[:, :KH], wq[:, KH:K2], wk[:, :KH], wk[:, KH:K2])):
        ws_v[n] = t
    wo_copy.wait()
    wg_copy.wait()
    wu_copy.wait()

    def phase1(i, carry):
        wd_copy(i).wait()

        def after(w, m):
            bits = pltpu.bitcast(m, jnp.int32) & zero_v[...]
            return pltpu.bitcast(pltpu.bitcast(w, jnp.int32) | bits, BF16)

        def block_sums(dst, b11, b12, b21, b22, m):
            for k, t in enumerate(_rhs_sums(after(b11, m).astype(F32), b12.astype(F32),
                                            b21.astype(F32), after(b22, m).astype(F32))):
                dst[k] = t

        def gu_sums(m, c):
            r0 = pl.multiple_of(i * 64, 64)
            r, r2, cs = pl.ds(r0, 64), pl.ds(KH + r0, 64), pl.ds(c * KH, KH)
            block_sums(gu_v.at[:, r, cs], wg_v[r, cs], wu_v[r, cs], wg_v[r2, cs], wu_v[r2, cs], m)

        def dn_sums(m, c):
            r = pl.ds(pl.multiple_of(i * (HF // NT) + c * 64, 64), 64)
            block_sums(dn_v.at[:, r], wd_v[0, r, :KH], wd_v[0, r, KH:K2], wd_v[1, r, :KH], wd_v[1, r, KH:K2], m)

        def wo_sums(m, c):
            r, r2 = pl.ds(pl.multiple_of(i * 64, 64), 64), pl.ds(pl.multiple_of(KH + i * 64, 64), 64)
            block_sums(os_v.at[:, r], wo_v[r, :KH], wo_v[r, KH:K2], wo_v[r2, :KH], wo_v[r2, KH:K2], m)

        jobs = [(wo_sums, 0)] * SWO + [(gu_sums, c) for c in range(F // KH)] + [(dn_sums, c) for c in range(HF // NT // 64)]

        def side(m, n0, n1):
            for n in range(n0, n1):
                r = (n - n0) * (D - 32) // max(n1 - n0 - 1, 1) // 8 * 8
                jobs[n][0](m[r:r + 32], jobs[n][1])

        def feature_map(p):
            return [_b(_dual_softmax(p[g * GW:(g + 1) * GW])) for g in range(NG)]

        ra = pl.ds(pl.multiple_of(i * TS, HM), HM)
        rb = pl.ds(pl.multiple_of(i * TS + HM, HM), HM)
        wk, wq = wt_v.at[1], wt_v.at[0]

        def cat(u, v):
            return jnp.concatenate([u, v], axis=1)

        m3 = _dot(wq[:, :KH], ys_v[i, 1], _NT)
        side(m3, 0, SP[0])
        t = _dot(wq[:, K2:], y_v[rb, K2:], _NT) + m3
        m5 = _dot(ws_v[2], y_v[rb, KH:K2], _NT)
        phiq_b = feature_map(t + m5)
        m4 = _dot(wk[:, KH:K2], ys_v[i, 2], _NT)
        side(m4, SP[0], SP[1])
        if ORD == 0:
            m1 = _dot(ws_v[0], ys_v[i, 0], _NT)
            side(m1, SP[1], len(jobs))
            phiq_a = feature_map(_dot(cat(ws_v[4], wq[:, K2:]), cat(ys_v[i, 4], y_v[ra, K2:]), _NT) + m1 + m4 - m5)
        t = _dot(wk[:, K2:], y_v[ra, K2:], _NT) + m4
        m2 = _dot(ws_v[1], y_v[ra, :KH], _NT)
        phik_a = feature_map(t + m2)
        if ORD == 1:
            m1 = _dot(ws_v[0], ys_v[i, 0], _NT)
            phiq_a = feature_map(_dot(cat(ws_v[4], wq[:, K2:]), cat(ys_v[i, 4], y_v[ra, K2:]), _NT) + m1 + m4 - m5)
        if ORD == 2:
            m1 = _dot(ws_v[0], ys_v[i, 0], _NT)
        phik_b = feature_map(_dot(cat(ws_v[3], wk[:, K2:]), cat(ys_v[i, 3], y_v[rb, K2:]), _NT) + m1 + m3 - m2)
        if ORD == 2:
            phiq_a = feature_map(_dot(cat(ws_v[4], wq[:, K2:]), cat(ys_v[i, 4], y_v[ra, K2:]), _NT) + m1 + m4 - m5)
        kv = [_dot(vt_v[i, g, :, :HM], phik_a[g], _NT) + kv_v[g] for g in range(NG)]
        kv = [_dot(vt_v[i, g, :, HM:], phik_b[g], _NT) + kv[g] for g in range(NG)]
        for g in range(NG):
            phiq_v[i, g, :, :HM] = phiq_a[g]
            phiq_v[i, g, :, HM:] = phiq_b[g]
            kv_v[g] = kv[g]
        return carry

    lax.fori_loop(0, NT, phase1, None)

    mr = _iota((MV, 2 * GW), 0)
    row_head = jnp.where(mr < GW, jnp.where(mr < DH, 0, 1), jnp.where(mr < GW + 4, 0, 1))
    same_head = row_head == (_iota((MV, 2 * GW), 1) & 1)
    for g in range(NG):
        kvb_v[g] = _b(jnp.where(same_head, kv_v[g], 0.0))

    def out_copy(i, half):
        rows = pl.ds(i * TS + half * HM, HM)
        return pltpu.make_async_copy(out_v.at[rows], out_hbm.at[rows], sem_o.at[2 * i + half])

    def phase2(i, carry):
        low = _iota((8, TS), 0) < 4
        ots = []
        for g in range(NG):
            nd = _dot(kvb_v[g], phiq_v[i, g])
            mixed = _recip(nd[GW:] + DEN_EPS)
            swapped = pltpu.roll(mixed, 4, 0)
            inv0 = jnp.where(low, mixed, swapped)
            inv1 = jnp.where(low, swapped, mixed)
            for j in range(GW // 8):
                inv = inv0 if 8 * (j + 1) <= DH else inv1 if 8 * j >= DH else mixed
                ots.append(nd[j * 8:(j + 1) * 8] * inv)
        ot = jnp.concatenate(ots, axis=0)
        ra = pl.ds(pl.multiple_of(i * TS, HM), HM)
        rb = pl.ds(pl.multiple_of(i * TS + HM, HM), HM)
        x1, x2 = x_v[ra, :].astype(F32), x_v[rb, :].astype(F32)
        if SWO == 0:
            h1 = x1 + _dot(_b(ot[:, :HM]), wo_v[...], _TN)
            y1 = _layernorm(h1)
            h2 = x2 + _dot(_b(ot[:, HM:]), wo_v[...], _TN)
            y2 = _layernorm(h2)
        else:
            o1, o2 = ot[:, :HM].T, ot[:, HM:].T
            s1, s2, s5, s6, s7 = _lhs_sums(o1[:, :KH], o1[:, KH:K2], o2[:, :KH], o2[:, KH:K2])
            o1, o2 = _b(o1), _b(o2)
            n1 = _dot(o1, wo_v[:, K2:]) + x1[:, K2:]
            m3 = _dot(o1[:, :KH], os_v[1])
            m5 = _dot(s5, wo_v[KH:K2, KH:K2])
            c12 = _dot(o1[:, K2:], wo_v[K2:, KH:K2]) + x1[:, KH:K2] + m3 + m5
            m4 = _dot(o2[:, KH:K2], os_v[2])
            m1 = _dot(s1, os_v[0])
            c11 = _dot(jnp.concatenate([s7, o1[:, K2:]], axis=1),
                       jnp.concatenate([os_v[4], wo_v[K2:, :KH]], axis=0)) + x1[:, :KH] + m1 + m4 - m5
            y1 = _layernorm(h1 := jnp.concatenate([c11, c12, n1], axis=1))
            n2 = _dot(o2, wo_v[:, K2:]) + x2[:, K2:]
            m2 = _dot(s2, wo_v[:KH, :KH])
            c21 = _dot(o2[:, K2:], wo_v[K2:, :KH]) + x2[:, :KH] + m2 + m4
            c22 = _dot(jnp.concatenate([s6, o2[:, K2:]], axis=1),
                       jnp.concatenate([os_v[3], wo_v[K2:, KH:K2]], axis=0)) + x2[:, KH:K2] + m1 + m3 - m2
            y2 = _layernorm(h2 := jnp.concatenate([c21, c22, n2], axis=1))

        cols = [slice(c * HF, (c + 1) * HF) for c in range(2)]
        a11, a22 = _b(y1[:, :KH]), _b(y2[:, KH:K2])
        m3s = [_dot(a11, gu_v[1, :, cols[c]]) for c in range(2)]
        s1, s2, s5, s6, s7 = _lhs_sums(y1[:, :KH], y1[:, KH:K2], y2[:, :KH], y2[:, KH:K2])
        r1, r2 = _b(y1[:, K2:]), _b(y2[:, K2:])
        ups = [_dot(r1, wu_v[K2:, cols[c]]) + m3s[c] for c in range(GU)]
        tops, bots = [], []
        for c in range(2):
            wgr, wur = wg_v[K2:, cols[c]], wu_v[K2:, cols[c]]
            m5 = _dot(s5, wu_v[KH:K2, cols[c]])
            up = ups[c] + m5 if c < GU else _dot(r1, wur) + m5 + m3s[c]
            m4 = _dot(a22, gu_v[2, :, cols[c]])
            m1 = _dot(s1, gu_v[0, :, cols[c]])
            gate = _dot(jnp.concatenate([s7, r1], axis=1),
                        jnp.concatenate([gu_v[4, :, cols[c]], wgr], axis=0)) + m1 + m4 - m5
            tops.append(_geglu(gate, up))
            m2 = _dot(s2, wg_v[:KH, cols[c]])
            gate = _dot(r2, wgr) + m2 + m4
            up = _dot(jnp.concatenate([s6, r2], axis=1),
                      jnp.concatenate([gu_v[3, :, cols[c]], wur], axis=0)) + m1 + m3s[c] - m2
            bots.append(_geglu(gate, up))

        s1, s2, s5, s6, s7 = _lhs_sums(tops[0], tops[1], bots[0], bots[1])
        a11, a12, a21, a22 = _b(tops[0]), _b(tops[1]), _b(bots[0]), _b(bots[1])
        m3 = _dot(a11, dn_v[1])
        m6 = _dot(s6, dn_v[3]) + h2[:, KH:K2]
        rem = (_dot(jnp.concatenate([a11, a21], axis=0), wd_v[0, :, K2:])
               + jnp.concatenate([h1[:, K2:], h2[:, K2:]], axis=0))
        m5 = _dot(s5, wd_v[1, :, KH:K2])
        r_top = _dot(a12, wd_v[1, :, K2:]) + rem[:HM]
        m4 = _dot(a22, dn_v[2])
        m1 = _dot(s1, dn_v[0])

        def emit(half, *blocks):
            rows = pl.ds(pl.multiple_of(i * TS + half * HM, HM), HM)
            out_v[rows, :] = jnp.concatenate(blocks, axis=1).astype(out_v.dtype)
            out_copy(i, half).start()

        c11 = _dot(s7, dn_v[4]) + h1[:, :KH] + m1 + m4 - m5
        emit(0, c11, h1[:, KH:K2] + m3 + m5, r_top)
        m2 = _dot(s2, wd_v[0, :, :KH])
        r_bot = _dot(a22, wd_v[1, :, K2:]) + rem[HM:]
        emit(1, h2[:, :KH] + m2 + m4, m6 + m1 + m3 - m2, r_bot)
        return carry

    lax.fori_loop(0, NT, phase2, None)
    for i in range(NT):
        for half in range(2):
            out_copy(i, half).wait()


@jax.jit
def pallas_sequential_preLN__linear_kernel_hedgehog__geglu_ffn__prompt_kernel(
    A_x: jax.Array,
    A_wqkv: jax.Array,
    A_w_phi: jax.Array,
    A_wo: jax.Array,
    B_x: jax.Array,
    B_w_gate: jax.Array,
    B_w_up: jax.Array,
    B_w_down: jax.Array,
):
    del B_x
    B, S, D = A_x.shape
    assert B == 1
    F = B_w_gate.shape[1]
    DH = D // H
    NG = H // 2
    GW = 2 * DH
    NT = S // TS
    hbm = pl.BlockSpec(memory_space=pl.ANY)
    out = pl.pallas_call(
        _kernel,
        out_shape=jax.ShapeDtypeStruct((S, D), A_x.dtype),
        in_specs=[hbm] * 7,
        out_specs=hbm,
        scratch_shapes=[
            pltpu.VMEM((S, D), BF16),
            pltpu.VMEM((3, D, D), BF16),
            pltpu.VMEM((DH, DH, H), BF16),
            pltpu.VMEM((D, D), BF16),
            pltpu.VMEM((D, F), BF16),
            pltpu.VMEM((D, F), BF16),
            pltpu.VMEM((2, F // 2, D), BF16),
            pltpu.VMEM((S, D), A_x.dtype),
            pltpu.VMEM((5, KH, F), BF16),
            pltpu.VMEM((5, F // 2, KH), BF16),
            pltpu.VMEM((5, KH, KH), BF16),
            pltpu.VMEM((3, D, D), BF16),
            pltpu.VMEM((5, D, KH), BF16),
            pltpu.VMEM((D // 128, 4 * GW, 128), BF16),
            pltpu.VMEM((S, D), BF16),
            pltpu.VMEM((NT, 5, HM, KH), BF16),
            pltpu.VMEM((NT, NG, GW + 8, TS), BF16),
            pltpu.VMEM((32, KH), jnp.int32),
            pltpu.VMEM((NT, NG, 2 * GW, TS), BF16),
            pltpu.VMEM((NG, GW + 8, 2 * GW), F32),
            pltpu.VMEM((NG, GW + 8, 2 * GW), BF16),
            pltpu.SemaphoreType.DMA((14 + 2 * NT,)),
            pltpu.SemaphoreType.DMA((2 * NT,)),
        ],
        compiler_params=pltpu.CompilerParams(vmem_limit_bytes=100 * 1024 * 1024),
    )(A_x.reshape(S, D), A_wqkv, jnp.transpose(A_w_phi, (1, 2, 0)), A_wo, B_w_gate, B_w_up,
      B_w_down.reshape(2, F // 2, D))
    return out.reshape(B, S, D)
```

```python
import math

import jax
import jax.numpy as jnp
from jax import lax
import jax.experimental.pallas as pl
import jax.experimental.pallas.tpu as pltpu

F32 = jnp.float32
BF16 = jnp.bfloat16

H = 32
LN_EPS = 1e-5
DEN_EPS = 1e-6
LOG2E = math.log2(math.e)

TS = 512
HM = TS // 2
KH = 256
K2 = 2 * KH
LNR = 32
WR = 64

_reciprocal = pltpu.reciprocal if hasattr(pltpu, "reciprocal") else pl.reciprocal
_NT = (((1,), (1,)), ((), ()))


def _dot(a, b):
    return jnp.dot(a, b, preferred_element_type=F32)


def _dot_nt(a, b):
    return lax.dot_general(a, b, _NT, preferred_element_type=F32)


def _b(t):
    return t.astype(BF16)


def _cat(*ts, axis=1):
    return jnp.concatenate(ts, axis=axis)


def _iota(shape, axis):
    return lax.broadcasted_iota(jnp.int32, shape, axis)


def _rows(start, n):
    return pl.ds(pl.multiple_of(start, n), n)


def _layernorm(x):
    out = []
    for r in range(0, x.shape[0], LNR):
        t = x[r:r + LNR].astype(F32)
        c = t - jnp.mean(t, axis=-1, keepdims=True)
        v = jnp.mean(c * c, axis=-1, keepdims=True)
        out.append(c * lax.rsqrt(v + LN_EPS))
    return jnp.concatenate(out, axis=0)


def _recip(s):
    r = _reciprocal(s, approx=True)
    return r * (2.0 - s * r)


def _reduce_f(rows, op):
    r = rows[0]
    for a in rows[1:]:
        r = op(r, a)
    r = op(r, pltpu.roll(r, 2, 0))
    return op(r, pltpu.roll(r, 4, 0))


def _dual_softmax(p):
    rows = [p[j * 8:(j + 1) * 8] for j in range(p.shape[0] // 8)]
    mx = _reduce_f(rows, jnp.maximum)
    mn = _reduce_f(rows, jnp.minimum)
    ep = [jnp.exp2(r - mx) for r in rows]
    en = [jnp.exp2(mn - r) for r in rows]
    rp = _recip(_reduce_f(ep, jnp.add))
    rn = _recip(_reduce_f(en, jnp.add))
    return jnp.concatenate([e * rp for e in ep] + [e * rn for e in en], axis=0)


def _gelu_tanh(g):
    c = math.sqrt(2.0 / math.pi)
    return (0.5 * g) * (1.0 + jnp.tanh(g * (c + (0.044715 * c) * (g * g))))


def _lhs_sums(a11, a12, a21, a22):
    return _b(a11 + a22), _b(a21 + a22), _b(a11 + a12), _b(a21 - a11), _b(a12 - a22)


def _rhs_sums(b11, b12, b21, b22):
    return _b(b11 + b22), _b(b12 - b22), _b(b21 - b11), _b(b11 + b12), _b(b21 + b22)


def _kernel(x_hbm, wqkv_hbm, wphi_hbm, wo_hbm, wg_hbm, wu_hbm, wd_hbm, out_hbm,
            x_v, wqkv_v, wphi_v, wo_v, wg_v, wu_v, wd_v, out_v,
            gu_v, dn_v, os_v, wt_v, ws_v, pt_v, y_v, ys_v, vt_v, phiq_v, kv_v, kvb_v, zero_v,
            sem_i, sem_o):
    S, D = x_v.shape
    HF = wg_v.shape[1] // 2
    DH = D // H
    NG = H // 2
    GW = 2 * DH
    MV = GW + 8
    NT = S // TS

    x_chunks = [(0, HM), (HM, HM)] + [(i * TS, TS) for i in range(1, NT)]
    nx = len(x_chunks)

    def x_copy(n):
        rows = pl.ds(*x_chunks[n])
        return pltpu.make_async_copy(x_hbm.at[rows], x_v.at[rows], sem_i.at[7 + n])

    def wqkv_copy(j):
        return pltpu.make_async_copy(wqkv_hbm.at[:, pl.ds(j * D, D)], wqkv_v.at[j], sem_i.at[j])

    def wd_copy(i):
        rows = pl.ds(i * (HF // NT), HF // NT)
        return pltpu.make_async_copy(wd_hbm.at[:, rows], wd_v.at[:, rows], sem_i.at[7 + nx + i])

    wo_copy = pltpu.make_async_copy(wo_hbm, wo_v, sem_i.at[3])
    wg_copy = pltpu.make_async_copy(wg_hbm, wg_v, sem_i.at[4])
    wu_copy = pltpu.make_async_copy(wu_hbm, wu_v, sem_i.at[5])
    wphi_copy = pltpu.make_async_copy(wphi_hbm, wphi_v, sem_i.at[6])

    wphi_copy.start()
    wqkv_copy(2).start()
    for n in range(nx):
        x_copy(n).start()
    wqkv_copy(1).start()
    wqkv_copy(0).start()
    wo_copy.start()
    wg_copy.start()
    wu_copy.start()
    for i in range(NT):
        wd_copy(i).start()

    src = _iota((D, 128), 0)
    dst = (src & (H - 1)) * DH + (src >> 5)
    lane = _iota((D, 128), 1)
    wphi_copy.wait()
    wcat = jnp.concatenate([wphi_v[d] for d in range(DH)], axis=1)
    BW = 4 * GW
    rr = _iota((BW, 128), 0)
    cc = _iota((BW, 128), 1)
    pair = rr // GW
    feat = (rr - pair * GW) >> 1
    first = (2 * pair + (rr & 1)) * DH
    expand = _b(jnp.where(feat == cc, 1.0, 0.0))[:, :DH]
    for j in range(D // 128):
        w2t = _b(_dot(wcat, _b(jnp.where(dst == lane + 128 * j, 1.0, 0.0))))
        d_of_col = cc + (128 - 3 * GW) * j - first
        pt_v[j] = _b(jnp.where((d_of_col >= 0) & (d_of_col < DH), _dot(expand, w2t), 0.0))
    kv_v[...] = jnp.zeros(kv_v.shape, F32)
    zero_v[...] = jnp.zeros(zero_v.shape, jnp.int32)

    def ln_half(r0):
        y = _layernorm(x_v[r0:r0 + HM, :])
        y_v[r0:r0 + HM, :] = _b(y)
        return y

    def store_sums(i, y1, y2):
        for n, t in enumerate(_rhs_sums(y1[:, :KH], y2[:, :KH], y1[:, KH:K2], y2[:, KH:K2])):
            ys_v[i, n] = t

    def v_proj(r0, y, c, nc):
        rows = y.shape[0]
        gs = NG // nc
        vt = _dot_nt(wt_v[2, c * gs * GW:(c + 1) * gs * GW, :], y)
        ones = jnp.ones((8, rows), F32)
        for g in range(gs):
            vt_v[r0 // TS, c * gs + g, :, r0 % TS:r0 % TS + rows] = _b(
                _cat(vt[g * GW:(g + 1) * GW], ones, axis=0))

    def fold(j):
        blocks, tail = [], None
        for c in range(D // 128):
            r = _dot_nt(pt_v[c], wqkv_v[j, :, 128 * c:128 * (c + 1)])
            blocks += [r[:GW] if tail is None else r[:GW] + tail, r[GW:3 * GW]]
            tail = r[3 * GW:]
        w = jnp.concatenate(blocks + [tail], axis=0) * LOG2E
        wt_v[j] = _b(w)
        return w

    wqkv_copy(2).wait()
    wt_v[2] = wqkv_v[2].T
    x_copy(0).wait()
    y1 = ln_half(0)
    x_copy(1).wait()
    v_proj(0, _b(y1), 0, 1)
    y2 = ln_half(HM)
    v_proj(HM, _b(y2), 0, 1)
    store_sums(0, y1, y2)
    for n in range(2, nx):
        x_copy(n).wait()
    y1, y2 = ln_half(TS), ln_half(TS + HM)
    store_sums(1, y1, y2)
    for i in range(2, NT):
        cur = _cat(_b(y1), _b(y2), axis=0)
        y1 = ln_half(i * TS)
        v_proj((i - 1) * TS, cur, 0, 2)
        y2 = ln_half(i * TS + HM)
        store_sums(i, y1, y2)
        v_proj((i - 1) * TS, cur, 1, 2)
    wqkv_copy(1).wait()
    wqkv_copy(0).wait()
    v_proj((NT - 1) * TS, _cat(_b(y1), _b(y2), axis=0), 0, 1)
    wk, wq = fold(1), fold(0)
    for n, t in enumerate(_lhs_sums(wq[:, :KH], wq[:, KH:K2], wk[:, :KH], wk[:, KH:K2])):
        ws_v[n] = t
    wo_copy.wait()
    wg_copy.wait()
    wu_copy.wait()

    def phase1(i, carry):
        wd_copy(i).wait()

        def after(w, m):
            bits = pltpu.bitcast(m, jnp.int32) & zero_v[...]
            return pltpu.bitcast(pltpu.bitcast(w, jnp.int32) | bits, BF16)

        def block_sums(dst, b11, b12, b21, b22, m):
            for n, t in enumerate(_rhs_sums(after(b11, m).astype(F32), b12.astype(F32),
                                            b21.astype(F32), after(b22, m).astype(F32))):
                dst[n] = t

        r1, r2 = _rows(i * WR, WR), _rows(KH + i * WR, WR)

        def wo_sums(m, c):
            block_sums(os_v.at[:, r1], wo_v[r1, :KH], wo_v[r1, KH:K2], wo_v[r2, :KH], wo_v[r2, KH:K2], m)

        def gu_sums(m, c):
            j, c = divmod(c, HF // KH)
            w_v, c1, c2 = (wg_v, wu_v)[j], pl.ds(c * KH, KH), pl.ds(HF + c * KH, KH)
            block_sums(gu_v.at[j, :, r1, c1], w_v[r1, c1], w_v[r1, c2], w_v[r2, c1], w_v[r2, c2], m)

        def dn_sums(m, c):
            r = _rows(i * (HF // NT) + c * WR, WR)
            block_sums(dn_v.at[:, r], wd_v[0, r, :KH], wd_v[0, r, KH:K2], wd_v[1, r, :KH], wd_v[1, r, KH:K2], m)

        jobs = ([(wo_sums, 0)] + [(gu_sums, c) for c in range(2 * HF // KH)]
                + [(dn_sums, c) for c in range(HF // NT // WR)])

        def weight_sums(m, n0, n1):
            for n in range(n0, n1):
                r = (n - n0) * (D - WR // 2) // (n1 - n0 - 1) // 8 * 8
                jobs[n][0](m[r:r + WR // 2], jobs[n][1])

        def feature_map(p):
            return [_b(_dual_softmax(p[g * GW:(g + 1) * GW])) for g in range(NG)]

        ya, yb = y_v.at[_rows(i * TS, HM)], y_v.at[_rows(i * TS + HM, HM)]
        wq, wk = wt_v.at[0], wt_v.at[1]
        m3 = _dot_nt(wq[:, :KH], ys_v[i, 1])
        weight_sums(m3, 0, 4)
        t = _dot_nt(wq[:, K2:], yb[:, K2:]) + m3
        m5 = _dot_nt(ws_v[2], yb[:, KH:K2])
        phiq_b = feature_map(t + m5)
        m4 = _dot_nt(wk[:, KH:K2], ys_v[i, 2])
        weight_sums(m4, 4, 8)
        m1 = _dot_nt(ws_v[0], ys_v[i, 0])
        weight_sums(m1, 8, len(jobs))
        phiq_a = feature_map(_dot_nt(_cat(ws_v[4], wq[:, K2:]), _cat(ys_v[i, 4], ya[:, K2:])) + m1 + m4 - m5)
        t = _dot_nt(wk[:, K2:], ya[:, K2:]) + m4
        m2 = _dot_nt(ws_v[1], ya[:, :KH])
        phik_a = feature_map(t + m2)
        phik_b = feature_map(_dot_nt(_cat(ws_v[3], wk[:, K2:]), _cat(ys_v[i, 3], yb[:, K2:])) + m1 + m3 - m2)
        kv = [_dot_nt(vt_v[i, g, :, :HM], phik_a[g]) + kv_v[g] for g in range(NG)]
        kv = [_dot_nt(vt_v[i, g, :, HM:], phik_b[g]) + kv[g] for g in range(NG)]
        for g in range(NG):
            phiq_v[i, g, :, :HM] = phiq_a[g]
            phiq_v[i, g, :, HM:] = phiq_b[g]
            kv_v[g] = kv[g]
        return carry

    lax.fori_loop(0, NT, phase1, None)

    mr = _iota((MV, 2 * GW), 0)
    row_head = jnp.where(mr < GW, jnp.where(mr < DH, 0, 1), jnp.where(mr < GW + 4, 0, 1))
    same_head = row_head == (_iota((MV, 2 * GW), 1) & 1)
    for g in range(NG):
        kvb_v[g] = _b(jnp.where(same_head, kv_v[g], 0.0))

    def out_copy(i, half):
        rows = pl.ds(i * TS + half * HM, HM)
        return pltpu.make_async_copy(out_v.at[rows], out_hbm.at[rows], sem_o.at[2 * i + half])

    def phase2(i, carry):
        low = _iota((8, TS), 0) < 4
        ots = []
        for g in range(NG):
            nd = _dot(kvb_v[g], phiq_v[i, g])
            mixed = _recip(nd[GW:] + DEN_EPS)
            swapped = pltpu.roll(mixed, 4, 0)
            inv0 = jnp.where(low, mixed, swapped)
            inv1 = jnp.where(low, swapped, mixed)
            for j in range(GW // 8):
                inv = inv0 if 8 * (j + 1) <= DH else inv1 if 8 * j >= DH else mixed
                ots.append(nd[j * 8:(j + 1) * 8] * inv)
        ot = jnp.concatenate(ots, axis=0)
        ra, rb = _rows(i * TS, HM), _rows(i * TS + HM, HM)
        x1, x2 = x_v[ra, :].astype(F32), x_v[rb, :].astype(F32)

        o1, o2 = ot[:, :HM].T, ot[:, HM:].T
        s1, s2, s5, s6, s7 = _lhs_sums(o1[:, :KH], o1[:, KH:K2], o2[:, :KH], o2[:, KH:K2])
        o1, o2 = _b(o1), _b(o2)
        n1 = _dot(o1, wo_v[:, K2:]) + x1[:, K2:]
        m3 = _dot(o1[:, :KH], os_v[1])
        m5 = _dot(s5, wo_v[KH:K2, KH:K2])
        c12 = _dot(o1[:, K2:], wo_v[K2:, KH:K2]) + x1[:, KH:K2] + m3 + m5
        m4 = _dot(o2[:, KH:K2], os_v[2])
        m1 = _dot(s1, os_v[0])
        c11 = _dot(_cat(s7, o1[:, K2:]), _cat(os_v[4], wo_v[K2:, :KH], axis=0)) + x1[:, :KH] + m1 + m4 - m5
        h1 = _cat(c11, c12, n1)
        y1 = _layernorm(h1)
        n2 = _dot(o2, wo_v[:, K2:]) + x2[:, K2:]
        m2 = _dot(s2, wo_v[:KH, :KH])
        c21 = _dot(o2[:, K2:], wo_v[K2:, :KH]) + x2[:, :KH] + m2 + m4
        c22 = _dot(_cat(s6, o2[:, K2:]), _cat(os_v[3], wo_v[K2:, KH:K2], axis=0)) + x2[:, KH:K2] + m1 + m3 - m2
        h2 = _cat(c21, c22, n2)
        y2 = _layernorm(h2)

        s1, s2, s5, s6, s7 = _lhs_sums(y1[:, :KH], y1[:, KH:K2], y2[:, :KH], y2[:, KH:K2])
        y1, y2 = _b(y1), _b(y2)
        m3s = [_dot(y1[:, :KH], gu_v[j, 1]) for j in range(2)]

        def hidden_steps(j, w_v, post, out):
            t = _dot(y1[:, K2:], w_v[K2:, HF:]) + m3s[j]
            yield
            m5 = _dot(s5, w_v[KH:K2, HF:])
            out[1] = post(1, t + m5)
            yield
            m4 = _dot(y2[:, KH:K2], gu_v[j, 2])
            yield
            m1 = _dot(s1, gu_v[j, 0])
            yield
            m7 = _dot(_cat(s7, y1[:, K2:]), _cat(gu_v[j, 4], w_v[K2:, :HF], axis=0))
            out[0] = post(0, m7 + m1 + m4 - m5)
            yield
            t = _dot(y2[:, K2:], w_v[K2:, :HF]) + m4
            yield
            m2 = _dot(s2, w_v[:KH, :HF])
            out[2] = post(2, t + m2)
            yield
            m6 = _dot(_cat(s6, y2[:, K2:]), _cat(gu_v[j, 3], w_v[K2:, HF:], axis=0))
            out[3] = post(3, m6 + m1 + m3s[j] - m2)
            yield

        gate, act = [None] * 4, [None] * 4
        for _ in zip(hidden_steps(0, wg_v, lambda n, g: _gelu_tanh(g), gate),
                     hidden_steps(1, wu_v, lambda n, u: gate[n] * u, act)):
            pass

        s1, s2, s5, s6, s7 = _lhs_sums(*act)
        a11, a12, a21, a22 = [_b(t) for t in act]
        wd_last = _cat(wd_v[0, :, K2:], wd_v[1, :, K2:], axis=0)

        def emit(half, rows, *blocks):
            out_v[rows, :] = _cat(*blocks).astype(out_v.dtype)
            out_copy(i, half).start()

        m3 = _dot(a11, dn_v[1])
        m5 = _dot(s5, wd_v[1, :, KH:K2])
        n1 = _dot(_cat(a11, a12), wd_last) + h1[:, K2:]
        m6 = _dot(s6, dn_v[3]) + h2[:, KH:K2]
        n2 = _dot(_cat(a21, a22), wd_last) + h2[:, K2:]
        m4 = _dot(a22, dn_v[2])
        m1 = _dot(s1, dn_v[0])
        c11 = _dot(s7, dn_v[4]) + h1[:, :KH] + m1 + m4 - m5
        emit(0, ra, c11, h1[:, KH:K2] + m3 + m5, n1)
        t1, t2 = h2[:, :KH] + m4, m6 + m1 + m3
        m2 = _dot(s2, wd_v[0, :, :KH])
        emit(1, rb, m2 + t1, t2 - m2, n2)
        return carry

    lax.fori_loop(0, NT, phase2, None)
    for i in range(NT):
        for half in range(2):
            out_copy(i, half).wait()


@jax.jit
def pallas_sequential_preLN__linear_kernel_hedgehog__geglu_ffn__prompt_kernel(
    A_x: jax.Array,
    A_wqkv: jax.Array,
    A_w_phi: jax.Array,
    A_wo: jax.Array,
    B_x: jax.Array,
    B_w_gate: jax.Array,
    B_w_up: jax.Array,
    B_w_down: jax.Array,
):
    del B_x
    B, S, D = A_x.shape
    F = B_w_gate.shape[1]
    assert (B, S, D, F) == (1, 2048, 640, 1536)
    DH = D // H
    NG = H // 2
    GW = 2 * DH
    NT = S // TS
    hbm = pl.BlockSpec(memory_space=pl.ANY)
    out = pl.pallas_call(
        _kernel,
        out_shape=jax.ShapeDtypeStruct((S, D), A_x.dtype),
        in_specs=[hbm] * 7,
        out_specs=hbm,
        scratch_shapes=[
            pltpu.VMEM((S, D), BF16),
            pltpu.VMEM((3, D, D), BF16),
            pltpu.VMEM((DH, DH, H), BF16),
            pltpu.VMEM((D, D), BF16),
            pltpu.VMEM((D, F), BF16),
            pltpu.VMEM((D, F), BF16),
            pltpu.VMEM((2, F // 2, D), BF16),
            pltpu.VMEM((S, D), A_x.dtype),
            pltpu.VMEM((2, 5, KH, F // 2), BF16),
            pltpu.VMEM((5, F // 2, KH), BF16),
            pltpu.VMEM((5, KH, KH), BF16),
            pltpu.VMEM((3, D, D), BF16),
            pltpu.VMEM((5, D, KH), BF16),
            pltpu.VMEM((D // 128, 4 * GW, 128), BF16),
            pltpu.VMEM((S, D), BF16),
            pltpu.VMEM((NT, 5, HM, KH), BF16),
            pltpu.VMEM((NT, NG, GW + 8, TS), BF16),
            pltpu.VMEM((NT, NG, 2 * GW, TS), BF16),
            pltpu.VMEM((NG, GW + 8, 2 * GW), F32),
            pltpu.VMEM((NG, GW + 8, 2 * GW), BF16),
            pltpu.VMEM((WR // 2, KH), jnp.int32),
            pltpu.SemaphoreType.DMA((8 + 2 * NT,)),
            pltpu.SemaphoreType.DMA((2 * NT,)),
        ],
        compiler_params=pltpu.CompilerParams(vmem_limit_bytes=100 * 1024 * 1024),
    )(A_x.reshape(S, D), A_wqkv, jnp.transpose(A_w_phi, (1, 2, 0)), A_wo, B_w_gate, B_w_up,
      B_w_down.reshape(2, F // 2, D))
    return out.reshape(B, S, D)
```

```python
import math

import jax
import jax.numpy as jnp
from jax import lax
import jax.experimental.pallas as pl
import jax.experimental.pallas.tpu as pltpu

F32 = jnp.float32
BF16 = jnp.bfloat16

H = 32
LN_EPS = 1e-5
DEN_EPS = 1e-6
LOG2E = math.log2(math.e)

TS = 512
HM = TS // 2
KH = 256
K2 = 2 * KH
LNR = 16
WR = 64

_reciprocal = pltpu.reciprocal if hasattr(pltpu, "reciprocal") else pl.reciprocal
_NT = (((1,), (1,)), ((), ()))


def _dot(a, b):
    return jnp.dot(a, b, preferred_element_type=F32)


def _dot_nt(a, b):
    return lax.dot_general(a, b, _NT, preferred_element_type=F32)


def _b(t):
    return t.astype(BF16)


def _cat(*ts, axis=1):
    return jnp.concatenate(ts, axis=axis)


def _iota(shape, axis):
    return lax.broadcasted_iota(jnp.int32, shape, axis)


def _rows(start, n):
    return pl.ds(start if isinstance(start, int) else pl.multiple_of(start, n), n)


def _layernorm(x):
    out = []
    for r in range(0, x.shape[0], LNR):
        t = x[r:r + LNR].astype(F32)
        c = t - jnp.mean(t, axis=-1, keepdims=True)
        v = jnp.mean(c * c, axis=-1, keepdims=True)
        out.append(c * lax.rsqrt(v + LN_EPS))
    return jnp.concatenate(out, axis=0)


def _recip(s):
    r = _reciprocal(s, approx=True)
    return r * (2.0 - s * r)


def _reduce_f(rows, op):
    r = rows[0]
    for a in rows[1:]:
        r = op(r, a)
    r = op(r, pltpu.roll(r, 2, 0))
    return op(r, pltpu.roll(r, 4, 0))


def _dual_softmax(p):
    rows = [p[j * 8:(j + 1) * 8] for j in range(p.shape[0] // 8)]
    mx = _reduce_f(rows, jnp.maximum)
    mn = _reduce_f(rows, jnp.minimum)
    ep = [jnp.exp2(r - mx) for r in rows]
    en = [jnp.exp2(mn - r) for r in rows]
    rp = _recip(_reduce_f(ep, jnp.add))
    rn = _recip(_reduce_f(en, jnp.add))
    return jnp.concatenate([e * rp for e in ep] + [e * rn for e in en], axis=0)


def _gelu_tanh(g):
    c = math.sqrt(2.0 / math.pi)
    return (0.5 * g) * (1.0 + jnp.tanh(g * (c + (0.044715 * c) * (g * g))))


def _lhs_sums(a11, a12, a21, a22):
    return _b(a11 + a22), _b(a21 + a22), _b(a11 + a12), _b(a21 - a11), _b(a12 - a22)


def _rhs_sums(b11, b12, b21, b22):
    return _b(b11 + b22), _b(b12 - b22), _b(b21 - b11), _b(b11 + b12), _b(b21 + b22)


def _kernel(x_hbm, wqkv_hbm, wphi_hbm, wo_hbm, wg_hbm, wu_hbm, wd_hbm, out_hbm,
            x_v, wqkv_v, wphi_v, wo_v, wg_v, wu_v, wd_v, out_v,
            gu_v, dn_v, os_v, wt_v, ws_v, pt_v, y_v, ys_v, vt_v, phiq_v, kv_v, kvb_v, zero_v,
            sem_i, sem_o):
    S, D = x_v.shape
    HF = wg_v.shape[1] // 2
    DH = D // H
    NG = H // 2
    GW = 2 * DH
    MV = GW + 8
    NT = S // TS

    x_chunks = [(0, HM), (HM, HM)] + [(i * TS, TS) for i in range(1, NT)]
    nx = len(x_chunks)

    def x_copy(n):
        rows = pl.ds(*x_chunks[n])
        return pltpu.make_async_copy(x_hbm.at[rows], x_v.at[rows], sem_i.at[7 + n])

    def wqkv_copy(j):
        return pltpu.make_async_copy(wqkv_hbm.at[:, pl.ds(j * D, D)], wqkv_v.at[j], sem_i.at[j])

    def wd_copy(i):
        rows = pl.ds(i * (HF // NT), HF // NT)
        return pltpu.make_async_copy(wd_hbm.at[:, rows], wd_v.at[:, rows], sem_i.at[7 + nx + i])

    wo_copy = pltpu.make_async_copy(wo_hbm, wo_v, sem_i.at[3])
    wg_copy = pltpu.make_async_copy(wg_hbm, wg_v, sem_i.at[4])
    wu_copy = pltpu.make_async_copy(wu_hbm, wu_v, sem_i.at[5])
    wphi_copy = pltpu.make_async_copy(wphi_hbm, wphi_v, sem_i.at[6])

    wphi_copy.start()
    wqkv_copy(2).start()
    for n in range(nx):
        x_copy(n).start()
    wqkv_copy(1).start()
    wqkv_copy(0).start()
    wo_copy.start()
    wg_copy.start()
    wu_copy.start()
    for i in range(NT):
        wd_copy(i).start()

    src = _iota((D, 128), 0)
    dst = (src & (H - 1)) * DH + (src >> 5)
    lane = _iota((D, 128), 1)
    wphi_copy.wait()
    wcat = jnp.concatenate([wphi_v[d] for d in range(DH)], axis=1)
    BW = 4 * GW
    rr = _iota((BW, 128), 0)
    cc = _iota((BW, 128), 1)
    pair = rr // GW
    feat = (rr - pair * GW) >> 1
    first = (2 * pair + (rr & 1)) * DH
    expand = _b(jnp.where(feat == cc, 1.0, 0.0))[:, :DH]
    for j in range(D // 128):
        w2t = _b(_dot(wcat, _b(jnp.where(dst == lane + 128 * j, 1.0, 0.0))))
        d_of_col = cc + (128 - 3 * GW) * j - first
        pt_v[j] = _b(jnp.where((d_of_col >= 0) & (d_of_col < DH), _dot(expand, w2t), 0.0))
    kv_v[...] = jnp.zeros(kv_v.shape, F32)
    zero_v[...] = jnp.zeros(zero_v.shape, jnp.int32)

    def ln_half(r0):
        y = _layernorm(x_v[r0:r0 + HM, :])
        y_v[r0:r0 + HM, :] = _b(y)
        return y

    def store_sums(i, y1, y2):
        for n, t in enumerate(_rhs_sums(y1[:, :KH], y2[:, :KH], y1[:, KH:K2], y2[:, KH:K2])):
            ys_v[i, n] = t

    def v_proj(r0, y, c, nc):
        rows = y.shape[0]
        gs = NG // nc
        vt = _dot_nt(wt_v[2, c * gs * GW:(c + 1) * gs * GW, :], y)
        ones = jnp.ones((8, rows), F32)
        for g in range(gs):
            vt_v[r0 // TS, c * gs + g, :, r0 % TS:r0 % TS + rows] = _b(
                _cat(vt[g * GW:(g + 1) * GW], ones, axis=0))

    def fold(j):
        blocks, tail = [], None
        for c in range(D // 128):
            r = _dot_nt(pt_v[c], wqkv_v[j, :, 128 * c:128 * (c + 1)])
            blocks += [r[:GW] if tail is None else r[:GW] + tail, r[GW:3 * GW]]
            tail = r[3 * GW:]
        w = jnp.concatenate(blocks + [tail], axis=0) * LOG2E
        wt_v[j] = _b(w)
        return w

    wqkv_copy(2).wait()
    wt_v[2] = wqkv_v[2].T
    x_copy(0).wait()
    y1 = ln_half(0)
    x_copy(1).wait()
    v_proj(0, _b(y1), 0, 1)
    y2 = ln_half(HM)
    v_proj(HM, _b(y2), 0, 1)
    store_sums(0, y1, y2)
    for n in range(2, nx):
        x_copy(n).wait()
    y1, y2 = ln_half(TS), ln_half(TS + HM)
    store_sums(1, y1, y2)
    for i in range(2, NT):
        cur = _cat(_b(y1), _b(y2), axis=0)
        y1 = ln_half(i * TS)
        v_proj((i - 1) * TS, cur, 0, 2)
        y2 = ln_half(i * TS + HM)
        store_sums(i, y1, y2)
        v_proj((i - 1) * TS, cur, 1, 2)
    wqkv_copy(1).wait()
    wqkv_copy(0).wait()
    v_proj((NT - 1) * TS, _cat(_b(y1), _b(y2), axis=0), 0, 1)
    wk, wq = fold(1), fold(0)
    for n, t in enumerate(_lhs_sums(wq[:, :KH], wq[:, KH:K2], wk[:, :KH], wk[:, KH:K2])):
        ws_v[n] = t
    wo_copy.wait()
    wg_copy.wait()
    wu_copy.wait()

    def phase1(i, carry):
        wd_copy(i).wait()

        def after(w, m):
            bits = pltpu.bitcast(m, jnp.int32) & zero_v[...]
            return pltpu.bitcast(pltpu.bitcast(w, jnp.int32) | bits, BF16)

        def block_sums(dst, b11, b12, b21, b22, m):
            for n, t in enumerate(_rhs_sums(after(b11, m).astype(F32), b12.astype(F32),
                                            b21.astype(F32), after(b22, m).astype(F32))):
                dst[n] = t

        r1, r2 = _rows(i * WR, WR), _rows(KH + i * WR, WR)

        def wo_sums(m, c):
            block_sums(os_v.at[:, r1], wo_v[r1, :KH], wo_v[r1, KH:K2], wo_v[r2, :KH], wo_v[r2, KH:K2], m)

        def gu_sums(m, c):
            j, c = divmod(c, HF // KH)
            w_v, c1, c2 = (wg_v, wu_v)[j], pl.ds(c * KH, KH), pl.ds(HF + c * KH, KH)
            block_sums(gu_v.at[j, :, r1, c1], w_v[r1, c1], w_v[r1, c2], w_v[r2, c1], w_v[r2, c2], m)

        def dn_sums(m, c):
            r = _rows(i * (HF // NT) + c * WR, WR)
            block_sums(dn_v.at[:, r], wd_v[0, r, :KH], wd_v[0, r, KH:K2], wd_v[1, r, :KH], wd_v[1, r, KH:K2], m)

        jobs = ([(wo_sums, 0)] + [(gu_sums, c) for c in range(2 * HF // KH)]
                + [(dn_sums, c) for c in range(HF // NT // WR)])

        def weight_sums(m, n0, n1):
            for n in range(n0, n1):
                r = (n - n0) * (D - WR // 2) // (n1 - n0 - 1) // 8 * 8
                jobs[n][0](m[r:r + WR // 2], jobs[n][1])

        def feature_map(p):
            return [_b(_dual_softmax(p[g * GW:(g + 1) * GW])) for g in range(NG)]

        ya, yb = y_v.at[_rows(i * TS, HM)], y_v.at[_rows(i * TS + HM, HM)]
        wq, wk = wt_v.at[0], wt_v.at[1]
        m3 = _dot_nt(wq[:, :KH], ys_v[i, 1])
        weight_sums(m3, 0, 6)
        t = _dot_nt(wq[:, K2:], yb[:, K2:]) + m3
        m5 = _dot_nt(ws_v[2], yb[:, KH:K2])
        phiq_b = feature_map(t + m5)
        m4 = _dot_nt(wk[:, KH:K2], ys_v[i, 2])
        m1 = _dot_nt(ws_v[0], ys_v[i, 0])
        weight_sums(m1, 6, len(jobs))
        phiq_a = feature_map(_dot_nt(_cat(ws_v[4], wq[:, K2:]), _cat(ys_v[i, 4], ya[:, K2:])) + m1 + m4 - m5)
        t = _dot_nt(wk[:, K2:], ya[:, K2:]) + m4
        m2 = _dot_nt(ws_v[1], ya[:, :KH])
        phik_a = feature_map(t + m2)
        phik_b = feature_map(_dot_nt(_cat(ws_v[3], wk[:, K2:]), _cat(ys_v[i, 3], yb[:, K2:])) + m1 + m3 - m2)
        kv = [_dot_nt(vt_v[i, g, :, :HM], phik_a[g]) + kv_v[g] for g in range(NG)]
        kv = [_dot_nt(vt_v[i, g, :, HM:], phik_b[g]) + kv[g] for g in range(NG)]
        for g in range(NG):
            phiq_v[i, g, :, :HM] = phiq_a[g]
            phiq_v[i, g, :, HM:] = phiq_b[g]
            kv_v[g] = kv[g]
        return carry

    lax.fori_loop(0, NT, phase1, None)

    mr = _iota((MV, 2 * GW), 0)
    row_head = jnp.where(mr < GW, jnp.where(mr < DH, 0, 1), jnp.where(mr < GW + 4, 0, 1))
    same_head = row_head == (_iota((MV, 2 * GW), 1) & 1)
    for g in range(NG):
        kvb_v[g] = _b(jnp.where(same_head, kv_v[g], 0.0))

    def out_part(i, part):
        return (_rows(i * TS + (0, HM, 0)[part], HM), pl.ds(*((KH, D - KH), (0, D), (0, KH))[part]))

    def out_copy(i, part):
        where = out_part(i, part)
        return pltpu.make_async_copy(out_v.at[where], out_hbm.at[where], sem_o.at[3 * i + part])

    def phase2(i, carry):
        low = _iota((8, TS), 0) < 4
        ots = []
        for g in range(NG):
            nd = _dot(kvb_v[g], phiq_v[i, g])
            mixed = _recip(nd[GW:] + DEN_EPS)
            swapped = pltpu.roll(mixed, 4, 0)
            inv0 = jnp.where(low, mixed, swapped)
            inv1 = jnp.where(low, swapped, mixed)
            for j in range(GW // 8):
                inv = inv0 if 8 * (j + 1) <= DH else inv1 if 8 * j >= DH else mixed
                ots.append(nd[j * 8:(j + 1) * 8] * inv)
        ot = jnp.concatenate(ots, axis=0)
        ra, rb = _rows(i * TS, HM), _rows(i * TS + HM, HM)
        x1, x2 = x_v[ra, :].astype(F32), x_v[rb, :].astype(F32)

        o1, o2 = ot[:, :HM].T, ot[:, HM:].T
        s1, s2, s5, s6, s7 = _lhs_sums(o1[:, :KH], o1[:, KH:K2], o2[:, :KH], o2[:, KH:K2])
        o1, o2 = _b(o1), _b(o2)
        m3 = _dot(o1[:, :KH], os_v[1])
        m5 = _dot(s5, wo_v[KH:K2, KH:K2])
        c12 = _dot(o1[:, K2:], wo_v[K2:, KH:K2]) + x1[:, KH:K2] + m3 + m5
        m4 = _dot(o2[:, KH:K2], os_v[2])
        m1 = _dot(s1, os_v[0])
        c11 = _dot(_cat(s7, o1[:, K2:]), _cat(os_v[4], wo_v[K2:, :KH], axis=0)) + x1[:, :KH] + m1 + m4 - m5
        n1 = _dot(o1, wo_v[:, K2:]) + x1[:, K2:]
        h1 = _cat(c11, c12, n1)
        y1 = _layernorm(h1)
        m2 = _dot(s2, wo_v[:KH, :KH])
        c21 = _dot(o2[:, K2:], wo_v[K2:, :KH]) + x2[:, :KH] + m2 + m4
        c22 = _dot(_cat(s6, o2[:, K2:]), _cat(os_v[3], wo_v[K2:, KH:K2], axis=0)) + x2[:, KH:K2] + m1 + m3 - m2
        n2 = _dot(o2, wo_v[:, K2:]) + x2[:, K2:]
        h2 = _cat(c21, c22, n2)
        y2 = _layernorm(h2)

        s1, s2, s5, s6, s7 = _lhs_sums(y1[:, :KH], y1[:, KH:K2], y2[:, :KH], y2[:, KH:K2])
        y1, y2 = _b(y1), _b(y2)
        m3s = [_dot(y1[:, :KH], gu_v[j, 1]) for j in range(2)]

        def hidden_steps(j, w_v, post, out):
            t = _dot(y1[:, K2:], w_v[K2:, HF:]) + m3s[j]
            yield
            m5 = _dot(s5, w_v[KH:K2, HF:])
            out[1] = post(1, t + m5)
            yield
            m4 = _dot(y2[:, KH:K2], gu_v[j, 2])
            yield
            m1 = _dot(s1, gu_v[j, 0])
            yield
            m7 = _dot(_cat(s7, y1[:, K2:]), _cat(gu_v[j, 4], w_v[K2:, :HF], axis=0))
            out[0] = post(0, m7 + m1 + m4 - m5)
            yield
            t = _dot(y2[:, K2:], w_v[K2:, :HF]) + m4
            yield
            m2 = _dot(s2, w_v[:KH, :HF])
            out[2] = post(2, t + m2)
            yield
            m6 = _dot(_cat(s6, y2[:, K2:]), _cat(gu_v[j, 3], w_v[K2:, HF:], axis=0))
            out[3] = post(3, m6 + m1 + m3s[j] - m2)
            yield

        gate, act = [None] * 4, [None] * 4
        for _ in zip(hidden_steps(0, wg_v, lambda n, g: _gelu_tanh(g), gate),
                     hidden_steps(1, wu_v, lambda n, u: gate[n] * u, act)):
            pass

        s1, s2, s5, s6, s7 = _lhs_sums(*act)
        a11, a12, a21, a22 = [_b(t) for t in act]
        wd_last = _cat(wd_v[0, :, K2:], wd_v[1, :, K2:], axis=0)

        def emit(part, *blocks):
            out_v[out_part(i, part)] = _cat(*blocks).astype(out_v.dtype)
            out_copy(i, part).start()

        m3 = _dot(a11, dn_v[1])
        m5 = _dot(s5, wd_v[1, :, KH:K2])
        n1 = _dot(_cat(a11, a12), wd_last) + h1[:, K2:]
        emit(0, h1[:, KH:K2] + m3 + m5, n1)
        m6 = _dot(s6, dn_v[3]) + h2[:, KH:K2]
        n2 = _dot(_cat(a21, a22), wd_last) + h2[:, K2:]
        m4 = _dot(a22, dn_v[2])
        m1 = _dot(s1, dn_v[0])
        t1, t2 = h2[:, :KH] + m4, m6 + m1 + m3
        m2 = _dot(s2, wd_v[0, :, :KH])
        emit(1, m2 + t1, t2 - m2, n2)
        emit(2, _dot(s7, dn_v[4]) + h1[:, :KH] + m1 + m4 - m5)
        return carry

    lax.fori_loop(0, NT, phase2, None)
    for i in range(NT):
        for part in range(3):
            out_copy(i, part).wait()


@jax.jit
def pallas_sequential_preLN__linear_kernel_hedgehog__geglu_ffn__prompt_kernel(
    A_x: jax.Array,
    A_wqkv: jax.Array,
    A_w_phi: jax.Array,
    A_wo: jax.Array,
    B_x: jax.Array,
    B_w_gate: jax.Array,
    B_w_up: jax.Array,
    B_w_down: jax.Array,
):
    del B_x
    B, S, D = A_x.shape
    F = B_w_gate.shape[1]
    assert (B, S, D, F) == (1, 2048, 640, 1536)
    DH = D // H
    NG = H // 2
    GW = 2 * DH
    NT = S // TS
    hbm = pl.BlockSpec(memory_space=pl.ANY)
    out = pl.pallas_call(
        _kernel,
        out_shape=jax.ShapeDtypeStruct((S, D), A_x.dtype),
        in_specs=[hbm] * 7,
        out_specs=hbm,
        scratch_shapes=[
            pltpu.VMEM((S, D), BF16),
            pltpu.VMEM((3, D, D), BF16),
            pltpu.VMEM((DH, DH, H), BF16),
            pltpu.VMEM((D, D), BF16),
            pltpu.VMEM((D, F), BF16),
            pltpu.VMEM((D, F), BF16),
            pltpu.VMEM((2, F // 2, D), BF16),
            pltpu.VMEM((S, D), A_x.dtype),
            pltpu.VMEM((2, 5, KH, F // 2), BF16),
            pltpu.VMEM((5, F // 2, KH), BF16),
            pltpu.VMEM((5, KH, KH), BF16),
            pltpu.VMEM((3, D, D), BF16),
            pltpu.VMEM((5, D, KH), BF16),
            pltpu.VMEM((D // 128, 4 * GW, 128), BF16),
            pltpu.VMEM((S, D), BF16),
            pltpu.VMEM((NT, 5, HM, KH), BF16),
            pltpu.VMEM((NT, NG, GW + 8, TS), BF16),
            pltpu.VMEM((NT, NG, 2 * GW, TS), BF16),
            pltpu.VMEM((NG, GW + 8, 2 * GW), F32),
            pltpu.VMEM((NG, GW + 8, 2 * GW), BF16),
            pltpu.VMEM((WR // 2, KH), jnp.int32),
            pltpu.SemaphoreType.DMA((8 + 2 * NT,)),
            pltpu.SemaphoreType.DMA((3 * NT,)),
        ],
        compiler_params=pltpu.CompilerParams(vmem_limit_bytes=100 * 1024 * 1024),
    )(A_x.reshape(S, D), A_wqkv, jnp.transpose(A_w_phi, (1, 2, 0)), A_wo, B_w_gate, B_w_up,
      B_w_down.reshape(2, F // 2, D))
    return out.reshape(B, S, D)
```

```python
import math

import jax
import jax.numpy as jnp
from jax import lax
import jax.experimental.pallas as pl
import jax.experimental.pallas.tpu as pltpu

F32 = jnp.float32
BF16 = jnp.bfloat16

H = 32
LN_EPS = 1e-5
DEN_EPS = 1e-6
LOG2E = math.log2(math.e)

TS = 512
HM = TS // 2
KH = 256
K2 = 2 * KH
LNR = 16
WR = 64

_reciprocal = pltpu.reciprocal if hasattr(pltpu, "reciprocal") else pl.reciprocal
_NT = (((1,), (1,)), ((), ()))


def _dot(a, b):
    return jnp.dot(a, b, preferred_element_type=F32)


def _dot_nt(a, b):
    return lax.dot_general(a, b, _NT, preferred_element_type=F32)


def _b(t):
    return t.astype(BF16)


def _cat(*ts, axis=1):
    return jnp.concatenate(ts, axis=axis)


def _iota(shape, axis):
    return lax.broadcasted_iota(jnp.int32, shape, axis)


def _rows(start, n):
    return pl.ds(start if isinstance(start, int) else pl.multiple_of(start, n), n)


def _layernorm(x):
    out = []
    for r in range(0, x.shape[0], LNR):
        t = x[r:r + LNR].astype(F32)
        c = t - jnp.mean(t, axis=-1, keepdims=True)
        v = jnp.mean(c * c, axis=-1, keepdims=True)
        out.append(c * lax.rsqrt(v + LN_EPS))
    return jnp.concatenate(out, axis=0)


def _recip(s):
    r = _reciprocal(s, approx=True)
    return r * (2.0 - s * r)


def _reduce_f(rows, op):
    r = rows[0]
    for a in rows[1:]:
        r = op(r, a)
    r = op(r, pltpu.roll(r, 2, 0))
    return op(r, pltpu.roll(r, 4, 0))


def _dual_softmax(p):
    rows = [p[j * 8:(j + 1) * 8] for j in range(p.shape[0] // 8)]
    mx = _reduce_f(rows, jnp.maximum)
    mn = _reduce_f(rows, jnp.minimum)
    ep = [jnp.exp2(r - mx) for r in rows]
    en = [jnp.exp2(mn - r) for r in rows]
    rp = _recip(_reduce_f(ep, jnp.add))
    rn = _recip(_reduce_f(en, jnp.add))
    return jnp.concatenate([e * rp for e in ep] + [e * rn for e in en], axis=0)


def _gelu_tanh(g):
    c = math.sqrt(2.0 / math.pi)
    return (0.5 * g) * (1.0 + jnp.tanh(g * (c + (0.044715 * c) * (g * g))))


def _lhs_sums(a11, a12, a21, a22):
    return _b(a11 + a22), _b(a21 + a22), _b(a11 + a12), _b(a21 - a11), _b(a12 - a22)


def _rhs_sums(b11, b12, b21, b22):
    return _b(b11 + b22), _b(b12 - b22), _b(b21 - b11), _b(b11 + b12), _b(b21 + b22)


def _kernel(x_hbm, wqkv_hbm, wphi_hbm, wo_hbm, wg_hbm, wu_hbm, wd_hbm, out_hbm,
            x_v, wqkv_v, wphi_v, wo_v, wg_v, wu_v, wd_v, out_v,
            gu_v, dn_v, os_v, wt_v, ws_v, pt_v, y_v, ys_v, vt_v, phiq_v, kv_v, kvb_v, zero_v,
            sem_i, sem_o):
    S, D = x_v.shape
    HF = wg_v.shape[1] // 2
    DH = D // H
    NG = H // 2
    GW = 2 * DH
    MV = GW + 8
    NT = S // TS

    x_chunks = [(0, HM), (HM, HM)] + [(i * TS, TS) for i in range(1, NT)]
    nx = len(x_chunks)

    def x_copy(n):
        rows = pl.ds(*x_chunks[n])
        return pltpu.make_async_copy(x_hbm.at[rows], x_v.at[rows], sem_i.at[7 + n])

    def wqkv_copy(j):
        return pltpu.make_async_copy(wqkv_hbm.at[:, pl.ds(j * D, D)], wqkv_v.at[j], sem_i.at[j])

    def wd_copy(i):
        rows = pl.ds(i * (HF // NT), HF // NT)
        return pltpu.make_async_copy(wd_hbm.at[:, rows], wd_v.at[:, rows], sem_i.at[7 + nx + i])

    wo_copy = pltpu.make_async_copy(wo_hbm, wo_v, sem_i.at[3])
    wg_copy = pltpu.make_async_copy(wg_hbm, wg_v, sem_i.at[4])
    wu_copy = pltpu.make_async_copy(wu_hbm, wu_v, sem_i.at[5])
    wphi_copy = pltpu.make_async_copy(wphi_hbm, wphi_v, sem_i.at[6])

    wphi_copy.start()
    wqkv_copy(2).start()
    for n in range(nx):
        x_copy(n).start()
    wqkv_copy(1).start()
    wqkv_copy(0).start()
    wo_copy.start()
    wg_copy.start()
    wu_copy.start()
    for i in range(NT):
        wd_copy(i).start()

    src = _iota((D, 128), 0)
    dst = (src & (H - 1)) * DH + (src >> 5)
    lane = _iota((D, 128), 1)
    wphi_copy.wait()
    wcat = jnp.concatenate([wphi_v[d] for d in range(DH)], axis=1)
    BW = 4 * GW
    rr = _iota((BW, 128), 0)
    cc = _iota((BW, 128), 1)
    pair = rr // GW
    feat = (rr - pair * GW) >> 1
    first = (2 * pair + (rr & 1)) * DH
    expand = _b(jnp.where(feat == cc, 1.0, 0.0))[:, :DH]
    for j in range(D // 128):
        w2t = _b(_dot(wcat, _b(jnp.where(dst == lane + 128 * j, 1.0, 0.0))))
        d_of_col = cc + (128 - 3 * GW) * j - first
        pt_v[j] = _b(jnp.where((d_of_col >= 0) & (d_of_col < DH), _dot(expand, w2t), 0.0))
    kv_v[...] = jnp.zeros(kv_v.shape, F32)
    zero_v[...] = jnp.zeros(zero_v.shape, jnp.int32)

    def ln_half(r0):
        y = _layernorm(x_v[r0:r0 + HM, :])
        y_v[r0:r0 + HM, :] = _b(y)
        return y

    def store_sums(i, y1, y2):
        for n, t in enumerate(_rhs_sums(y1[:, :KH], y2[:, :KH], y1[:, KH:K2], y2[:, KH:K2])):
            ys_v[i, n] = t

    def v_proj(r0, rows, c, nc):
        gs = NG // nc
        vt = _dot_nt(wt_v[2, c * gs * GW:(c + 1) * gs * GW, :], y_v[r0:r0 + rows, :])
        ones = jnp.ones((8, rows), F32)
        for g in range(gs):
            vt_v[r0 // TS, c * gs + g, :, r0 % TS:r0 % TS + rows] = _b(
                _cat(vt[g * GW:(g + 1) * GW], ones, axis=0))

    def fold(j):
        blocks, tail = [], None
        for c in range(D // 128):
            r = _dot_nt(pt_v[c], wqkv_v[j, :, 128 * c:128 * (c + 1)])
            blocks += [r[:GW] if tail is None else r[:GW] + tail, r[GW:3 * GW]]
            tail = r[3 * GW:]
        w = jnp.concatenate(blocks + [tail], axis=0) * LOG2E
        wt_v[j] = _b(w)
        return w

    wqkv_copy(2).wait()
    wt_v[2] = wqkv_v[2].T
    x_copy(0).wait()
    y1 = ln_half(0)
    x_copy(1).wait()
    v_proj(0, HM, 0, 1)
    y2 = ln_half(HM)
    v_proj(HM, HM, 0, 1)
    store_sums(0, y1, y2)
    for n in range(2, nx):
        x_copy(n).wait()
    y1, y2 = ln_half(TS), ln_half(TS + HM)
    store_sums(1, y1, y2)
    for i in range(2, NT):
        y1 = ln_half(i * TS)
        v_proj((i - 1) * TS, TS, 0, 2)
        y2 = ln_half(i * TS + HM)
        store_sums(i, y1, y2)
        v_proj((i - 1) * TS, TS, 1, 2)
    wqkv_copy(1).wait()
    wqkv_copy(0).wait()
    v_proj((NT - 1) * TS, TS, 0, 1)
    wk, wq = fold(1), fold(0)
    for n, t in enumerate(_lhs_sums(wq[:, :KH], wq[:, KH:K2], wk[:, :KH], wk[:, KH:K2])):
        ws_v[n] = t
    wo_copy.wait()
    wg_copy.wait()
    wu_copy.wait()

    def phase1(i, carry):
        wd_copy(i).wait()

        def after(w, m):
            bits = pltpu.bitcast(m, jnp.int32) & zero_v[...]
            return pltpu.bitcast(pltpu.bitcast(w, jnp.int32) | bits, BF16)

        def block_sums(dst, b11, b12, b21, b22, m):
            for n, t in enumerate(_rhs_sums(after(b11, m).astype(F32), b12.astype(F32),
                                            b21.astype(F32), after(b22, m).astype(F32))):
                dst[n] = t

        r1, r2 = _rows(i * WR, WR), _rows(KH + i * WR, WR)

        def wo_sums(m, c):
            block_sums(os_v.at[:, r1], wo_v[r1, :KH], wo_v[r1, KH:K2], wo_v[r2, :KH], wo_v[r2, KH:K2], m)

        def gu_sums(m, c):
            j, c = divmod(c, HF // KH)
            w_v, c1, c2 = (wg_v, wu_v)[j], pl.ds(c * KH, KH), pl.ds(HF + c * KH, KH)
            block_sums(gu_v.at[j, :, r1, c1], w_v[r1, c1], w_v[r1, c2], w_v[r2, c1], w_v[r2, c2], m)

        def dn_sums(m, c):
            r = _rows(i * (HF // NT) + c * WR, WR)
            block_sums(dn_v.at[:, r], wd_v[0, r, :KH], wd_v[0, r, KH:K2], wd_v[1, r, :KH], wd_v[1, r, KH:K2], m)

        jobs = ([(wo_sums, 0)] + [(gu_sums, c) for c in range(2 * HF // KH)]
                + [(dn_sums, c) for c in range(HF // NT // WR)])

        def weight_sums(m, n0, n1):
            for n in range(n0, n1):
                r = (n - n0) * (D - WR // 2) // (n1 - n0 - 1) // 8 * 8
                jobs[n][0](m[r:r + WR // 2], jobs[n][1])

        def feature_map(p):
            return [_b(_dual_softmax(p[g * GW:(g + 1) * GW])) for g in range(NG)]

        ya, yb = y_v.at[_rows(i * TS, HM)], y_v.at[_rows(i * TS + HM, HM)]
        wq, wk = wt_v.at[0], wt_v.at[1]
        m3 = _dot_nt(wq[:, :KH], ys_v[i, 1])
        weight_sums(m3, 0, 6)
        t = _dot_nt(wq[:, K2:], yb[:, K2:]) + m3
        m5 = _dot_nt(ws_v[2], yb[:, KH:K2])
        phiq_b = feature_map(t + m5)
        m4 = _dot_nt(wk[:, KH:K2], ys_v[i, 2])
        m1 = _dot_nt(ws_v[0], ys_v[i, 0])
        weight_sums(m1, 6, len(jobs))
        phiq_a = feature_map(_dot_nt(_cat(ws_v[4], wq[:, K2:]), _cat(ys_v[i, 4], ya[:, K2:])) + m1 + m4 - m5)
        t = _dot_nt(wk[:, K2:], ya[:, K2:]) + m4
        m2 = _dot_nt(ws_v[1], ya[:, :KH])
        phik_a = feature_map(t + m2)
        phik_b = feature_map(_dot_nt(_cat(ws_v[3], wk[:, K2:]), _cat(ys_v[i, 3], yb[:, K2:])) + m1 + m3 - m2)
        kv = [_dot_nt(vt_v[i, g, :, :HM], phik_a[g]) + kv_v[g] for g in range(NG)]
        kv = [_dot_nt(vt_v[i, g, :, HM:], phik_b[g]) + kv[g] for g in range(NG)]
        for g in range(NG):
            phiq_v[i, g, :, :HM] = phiq_a[g]
            phiq_v[i, g, :, HM:] = phiq_b[g]
            kv_v[g] = kv[g]
        return carry

    lax.fori_loop(0, NT, phase1, None)

    mr = _iota((MV, 2 * GW), 0)
    row_head = jnp.where(mr < GW, jnp.where(mr < DH, 0, 1), jnp.where(mr < GW + 4, 0, 1))
    same_head = row_head == (_iota((MV, 2 * GW), 1) & 1)
    for g in range(NG):
        kvb_v[g] = _b(jnp.where(same_head, kv_v[g], 0.0))

    def out_part(i, part):
        return (_rows(i * TS + (0, HM, 0)[part], HM), pl.ds(*((KH, D - KH), (0, D), (0, KH))[part]))

    def out_copy(i, part):
        where = out_part(i, part)
        return pltpu.make_async_copy(out_v.at[where], out_hbm.at[where], sem_o.at[3 * i + part])

    def phase2(i, carry):
        low = _iota((8, TS), 0) < 4
        ots = []
        for g in range(NG):
            nd = _dot(kvb_v[g], phiq_v[i, g])
            mixed = _recip(nd[GW:] + DEN_EPS)
            swapped = pltpu.roll(mixed, 4, 0)
            inv0 = jnp.where(low, mixed, swapped)
            inv1 = jnp.where(low, swapped, mixed)
            for j in range(GW // 8):
                inv = inv0 if 8 * (j + 1) <= DH else inv1 if 8 * j >= DH else mixed
                ots.append(nd[j * 8:(j + 1) * 8] * inv)
        ot = jnp.concatenate(ots, axis=0)
        ra, rb = _rows(i * TS, HM), _rows(i * TS + HM, HM)
        x1, x2 = x_v[ra, :].astype(F32), x_v[rb, :].astype(F32)

        o1, o2 = ot[:, :HM].T, ot[:, HM:].T
        s1, s2, s5, s6, s7 = _lhs_sums(o1[:, :KH], o1[:, KH:K2], o2[:, :KH], o2[:, KH:K2])
        o1, o2 = _b(o1), _b(o2)
        m3 = _dot(o1[:, :KH], os_v[1])
        m5 = _dot(s5, wo_v[KH:K2, KH:K2])
        c12 = _dot(o1[:, K2:], wo_v[K2:, KH:K2]) + x1[:, KH:K2] + m3 + m5
        m4 = _dot(o2[:, KH:K2], os_v[2])
        m1 = _dot(s1, os_v[0])
        c11 = _dot(_cat(s7, o1[:, K2:]), _cat(os_v[4], wo_v[K2:, :KH], axis=0)) + x1[:, :KH] + m1 + m4 - m5
        n1 = _dot(o1, wo_v[:, K2:]) + x1[:, K2:]
        h1 = _cat(c11, c12, n1)
        y1 = _layernorm(h1)
        m2 = _dot(s2, wo_v[:KH, :KH])
        c21 = _dot(o2[:, K2:], wo_v[K2:, :KH]) + x2[:, :KH] + m2 + m4
        c22 = _dot(_cat(s6, o2[:, K2:]), _cat(os_v[3], wo_v[K2:, KH:K2], axis=0)) + x2[:, KH:K2] + m1 + m3 - m2
        n2 = _dot(o2, wo_v[:, K2:]) + x2[:, K2:]
        h2 = _cat(c21, c22, n2)
        y2 = _layernorm(h2)

        s1, s2, s5, s6, s7 = _lhs_sums(y1[:, :KH], y1[:, KH:K2], y2[:, :KH], y2[:, KH:K2])
        y1, y2 = _b(y1), _b(y2)
        m3s = [_dot(y1[:, :KH], gu_v[j, 1]) for j in range(2)]

        def hidden_steps(j, w_v, post, out):
            t = _dot(y1[:, K2:], w_v[K2:, HF:]) + m3s[j]
            yield
            m5 = _dot(s5, w_v[KH:K2, HF:])
            out[1] = post(1, t + m5)
            yield
            m4 = _dot(y2[:, KH:K2], gu_v[j, 2])
            yield
            m1 = _dot(s1, gu_v[j, 0])
            yield
            m7 = _dot(_cat(s7, y1[:, K2:]), _cat(gu_v[j, 4], w_v[K2:, :HF], axis=0))
            out[0] = post(0, m7 + m1 + m4 - m5)
            yield
            t = _dot(y2[:, K2:], w_v[K2:, :HF]) + m4
            yield
            m2 = _dot(s2, w_v[:KH, :HF])
            out[2] = post(2, t + m2)
            yield
            m6 = _dot(_cat(s6, y2[:, K2:]), _cat(gu_v[j, 3], w_v[K2:, HF:], axis=0))
            out[3] = post(3, m6 + m1 + m3s[j] - m2)
            yield

        gate, act = [None] * 4, [None] * 4
        for _ in zip(hidden_steps(0, wg_v, lambda n, g: _gelu_tanh(g), gate),
                     hidden_steps(1, wu_v, lambda n, u: gate[n] * u, act)):
            pass

        s1, s2, s5, s6, s7 = _lhs_sums(*act)
        a11, a12, a21, a22 = [_b(t) for t in act]
        wd_last = _cat(wd_v[0, :, K2:], wd_v[1, :, K2:], axis=0)

        def emit(part, *blocks):
            out_v[out_part(i, part)] = _cat(*blocks).astype(out_v.dtype)
            out_copy(i, part).start()

        m3 = _dot(a11, dn_v[1])
        m5 = _dot(s5, wd_v[1, :, KH:K2])
        n1 = _dot(_cat(a11, a12), wd_last) + h1[:, K2:]
        emit(0, h1[:, KH:K2] + m3 + m5, n1)
        m6 = _dot(s6, dn_v[3]) + h2[:, KH:K2]
        n2 = _dot(_cat(a21, a22), wd_last) + h2[:, K2:]
        m4 = _dot(a22, dn_v[2])
        m1 = _dot(s1, dn_v[0])
        t1, t2 = h2[:, :KH] + m4, m6 + m1 + m3
        m2 = _dot(s2, wd_v[0, :, :KH])
        emit(1, m2 + t1, t2 - m2, n2)
        emit(2, _dot(s7, dn_v[4]) + h1[:, :KH] + m1 + m4 - m5)
        return carry

    lax.fori_loop(0, NT, phase2, None)
    for i in range(NT):
        for part in range(3):
            out_copy(i, part).wait()


@jax.jit
def pallas_sequential_preLN__linear_kernel_hedgehog__geglu_ffn__prompt_kernel(
    A_x: jax.Array,
    A_wqkv: jax.Array,
    A_w_phi: jax.Array,
    A_wo: jax.Array,
    B_x: jax.Array,
    B_w_gate: jax.Array,
    B_w_up: jax.Array,
    B_w_down: jax.Array,
):
    del B_x
    B, S, D = A_x.shape
    F = B_w_gate.shape[1]
    assert (B, S, D, F) == (1, 2048, 640, 1536)
    DH = D // H
    NG = H // 2
    GW = 2 * DH
    NT = S // TS
    hbm = pl.BlockSpec(memory_space=pl.ANY)
    out = pl.pallas_call(
        _kernel,
        out_shape=jax.ShapeDtypeStruct((S, D), A_x.dtype),
        in_specs=[hbm] * 7,
        out_specs=hbm,
        scratch_shapes=[
            pltpu.VMEM((S, D), BF16),
            pltpu.VMEM((3, D, D), BF16),
            pltpu.VMEM((DH, DH, H), BF16),
            pltpu.VMEM((D, D), BF16),
            pltpu.VMEM((D, F), BF16),
            pltpu.VMEM((D, F), BF16),
            pltpu.VMEM((2, F // 2, D), BF16),
            pltpu.VMEM((S, D), A_x.dtype),
            pltpu.VMEM((2, 5, KH, F // 2), BF16),
            pltpu.VMEM((5, F // 2, KH), BF16),
            pltpu.VMEM((5, KH, KH), BF16),
            pltpu.VMEM((3, D, D), BF16),
            pltpu.VMEM((5, D, KH), BF16),
            pltpu.VMEM((D // 128, 4 * GW, 128), BF16),
            pltpu.VMEM((S, D), BF16),
            pltpu.VMEM((NT, 5, HM, KH), BF16),
            pltpu.VMEM((NT, NG, GW + 8, TS), BF16),
            pltpu.VMEM((NT, NG, 2 * GW, TS), BF16),
            pltpu.VMEM((NG, GW + 8, 2 * GW), F32),
            pltpu.VMEM((NG, GW + 8, 2 * GW), BF16),
            pltpu.VMEM((WR // 2, KH), jnp.int32),
            pltpu.SemaphoreType.DMA((8 + 2 * NT,)),
            pltpu.SemaphoreType.DMA((3 * NT,)),
        ],
        compiler_params=pltpu.CompilerParams(vmem_limit_bytes=100 * 1024 * 1024),
    )(A_x.reshape(S, D), A_wqkv, jnp.transpose(A_w_phi, (1, 2, 0)), A_wo, B_w_gate, B_w_up,
      B_w_down.reshape(2, F // 2, D))
    return out.reshape(B, S, D)
```
